```python
import os as _os
_os.environ.setdefault("JAX_PLATFORMS", "cpu")
import jax
import jax.numpy as jnp

def _softmax(x, axis=-1):
    return jax.nn.softmax(x, axis=axis)
def _gelu(x):
    return jax.nn.gelu(x, approximate=True)
def _silu(x):
    return jax.nn.silu(x)
def _sigmoid(x):
    return jax.nn.sigmoid(x)
def _layernorm(x, axis=-1, eps=1e-5):
    m = jnp.mean(x, axis=axis, keepdims=True)
    v = jnp.var(x, axis=axis, keepdims=True)
    return (x - m) / jnp.sqrt(v + eps)
def _scatter_add(tgt, idx, src, axis=0):
    return tgt.at[idx].add(src)
def _segment_sum(src, seg, n):
    return jax.ops.segment_sum(src, seg, n)
class _Rng:
    def __init__(self, key):
        self._k = key
    def _next(self):
        self._k, sub = jax.random.split(self._k)
        return sub
    def normal(self, shape):
        return jax.random.normal(self._next(), shape, dtype=jnp.bfloat16)
    def randint(self, lo, hi, shape):
        return jax.random.randint(self._next(), shape, lo, hi, dtype=jnp.int32)
    def uniform(self, shape, lo=0.0, hi=1.0):
        return jax.random.uniform(self._next(), shape, jnp.bfloat16, lo, hi)
    def permutation(self, n):
        return jax.random.permutation(self._next(), n)


kernel_name = 'concat_heads__gqa_block_cached__mha_block_cached__near_ridge'

def setup_inputs():
    _rng = _Rng(jax.random.key(int.from_bytes(__import__("os").urandom(4), "little")))
    _w = (lambda a: (lambda t: t.astype(jnp.bfloat16) if jnp.issubdtype(t.dtype, jnp.floating) else t)(jnp.asarray(a)))
    def _A_setup():
        B, Sq, D = 16, 32, 512
        Hq, Hkv, Sk, Dh = 32, 8, 512, 128
        assert Hq % Hkv == 0, (Hq, Hkv)
        return {
            "x": _w((lambda *s: _rng.normal(s) * 0.8)(B, Sq, D)),
            "k_cache": _w((lambda *s: _rng.normal(s) * 0.8)(B, Hkv, Sk, Dh)),
            "v_cache": _w((lambda *s: _rng.normal(s) * 0.05)(B, Hkv, Sk, Dh)),
            "wq": _w((lambda *s: _rng.normal(s) * 0.8)(D, Hq * Dh) * (D ** -0.5)),
            "wo": _w((lambda *s: _rng.normal(s) * 0.05)(Hq * Dh, D) * ((Hq * Dh) ** -0.5)),
        }
    _A_in = _A_setup()

    def _B_setup():
        B, Sq, D = 16, 32, 512
        H, Sk, Dh = 32, 512, 128
        return {
            "x": _w((lambda *s: _rng.normal(s) * 0.8)(B, Sq, D)),
            "k_cache": _w((lambda *s: _rng.normal(s) * 0.8)(B, H, Sk, Dh)),
            "v_cache": _w((lambda *s: _rng.normal(s) * 0.05)(B, H, Sk, Dh)),
            "wq": _w((lambda *s: _rng.normal(s) * 0.8)(D, H * Dh) * (D ** -0.5)),
            "wo": _w((lambda *s: _rng.normal(s) * 0.05)(H * Dh, D) * ((H * Dh) ** -0.5)),
        }
    _B_in = _B_setup()

    return {
        "A_x": _A_in["x"],
        "A_k_cache": _A_in["k_cache"],
        "A_v_cache": _A_in["v_cache"],
        "A_wq": _A_in["wq"],
        "A_wo": _A_in["wo"],
        "B_x": _B_in["x"],
        "B_k_cache": _B_in["k_cache"],
        "B_v_cache": _B_in["v_cache"],
        "B_wq": _B_in["wq"],
        "B_wo": _B_in["wo"],
    }

def reference(A_x, A_k_cache, A_v_cache, A_wq, A_wo, B_x, B_k_cache, B_v_cache, B_wq, B_wo):
    def _A_ref(x, k_cache, v_cache, wq, wo):
        B, Sq, D = x.shape
        Hq, Dh = 32, 128
        Hkv = k_cache.shape[1]
        rep = Hq // Hkv
        q = (lambda x, *d: x.transpose(*d))((x @ wq).reshape(B, Sq, Hq, Dh), 0, 2, 1, 3)
        k = jnp.repeat(k_cache, rep, axis=1)
        v = jnp.repeat(v_cache, rep, axis=1)
        scores = jnp.einsum("bhqd,bhkd->bhqk", q, k) * (Dh ** -0.5)
        p = _softmax(scores, axis=-1)
        o = jnp.einsum("bhqk,bhkd->bhqd", p, v)
        return (lambda x, *d: x.transpose(*d))(o, 0, 2, 1, 3).reshape(B, Sq, Hq * Dh) @ wo

    def _B_ref(x, k_cache, v_cache, wq, wo):
        B, Sq, D = x.shape
        H, Dh = 32, 128
        q = (lambda x, *d: x.transpose(*d))((x @ wq).reshape(B, Sq, H, Dh), 0, 2, 1, 3)
        scores = jnp.einsum("bhqd,bhkd->bhqk", q, k_cache) * (Dh ** -0.5)
        p = _softmax(scores, axis=-1)
        o = jnp.einsum("bhqk,bhkd->bhqd", p, v_cache)
        return (lambda x, *d: x.transpose(*d))(o, 0, 2, 1, 3).reshape(B, Sq, H * Dh) @ wo

    a = _A_ref(A_x, A_k_cache, A_v_cache, A_wq, A_wo)
    b = _B_ref(B_x, B_k_cache, B_v_cache, B_wq, B_wo)
    return jnp.concatenate([a, b], axis=-1)
```

```python
import functools
import jax, jax.numpy as jnp, numpy as np
from jax import lax
from jax.experimental import pallas as pl
from jax.experimental.pallas import tpu as pltpu

NB, SQ, D, DH, SK = 16, 32, 512, 128, 512
NG = 8
GB = 4
NJ = NB // GB
NSTEP = NG * NJ
ROWS = GB * SQ
QSCALE = float(DH ** -0.5 * np.log2(np.e))
NSLOT = 3
PR = 128

def make(dma=True, compute=True, flags=None, order="c16", cuts=(0, 22, 55, 88, 110, 154, 176), wmode="col"):
    def kernel(ax, ak, av, awq, awo, bx, bk, bv, bwq, bwo, out,
               xbuf, w, kva, kvb, acc, ostage, asem, bsem, wsem, xsem, osem):
        kva32 = kva.bitcast(jnp.uint32); kvb32 = kvb.bitcast(jnp.uint32)
        def weight_copies(g, quarter):
            cs = []
            c0 = pl.multiple_of(g * 512, 512)
            for i in range(4):
                r = pl.multiple_of(quarter * 128 + i * 32, 32)
                for t, (sq, so) in enumerate(((awq, awo), (bwq, bwo))):
                    cs.append(pltpu.make_async_copy(sq.at[pl.ds(r, 32), pl.ds(c0, 512)], w.at[g, t, pl.ds(r, 32)], wsem.at[g]))
                    cs.append(pltpu.make_async_copy(so.at[pl.ds(c0 + r, 32)], w.at[g, 2 + t, pl.ds(r, 32)], wsem.at[g]))
            return cs
        def kv_items():
            A = [("a", t, i, 0, c) for c in range(4) for i in range(GB) for t in range(2)]
            if order == "c16":
                cc = [(hh, c) for hh in range(4) for c in range(4)]
            elif order == "h4":
                cc = [(hh, c) for c in range(4) for hh in range(4)]
            B = [("b", t, i, hh, c) for (hh, c) in cc for i in range(GB) for t in range(2)]
            items = []
            for n in range(32):
                items += B[4 * n:4 * n + 4] + [A[n]]
            return items
        ITEMS = kv_items()
        def kv_copy(item, g, j, slot):
            kind, t, i, hh, c = item
            b = j * GB + i
            if kind == "a":
                return pltpu.make_async_copy((ak, av)[t].at[b, g, pl.ds(c * PR, PR)], kva.at[slot, t, i, pl.ds(c * PR, PR)], asem.at[slot])
            return pltpu.make_async_copy((bk, bv)[t].at[b, 4 * g + hh, pl.ds(c * PR, PR)], kvb.at[slot, t, i, hh, pl.ds(c * PR, PR)], bsem.at[slot])
        def issue(step, lo, hi, static_step=False):
            if not dma or lo == hi: return
            g = step // NJ; j = step % NJ; slot = step % NSLOT
            def go(with_w):
                wc = weight_copies(g + 1, j) if with_w else None
                n = lo
                for e in range(lo, hi):
                    if e % 11 == 10:
                        if with_w:
                            wc[e // 11].start(priority=n % 2); n += 1
                    else:
                        kv_copy(ITEMS[e - e // 11], g, j, slot).start(priority=n % 2); n += 1
                if with_w:
                    for c in wc: c._used = True
            if static_step:
                go(True)
            else:
                @pl.when(step < NSTEP - NJ)
                def _(): go(True)
                @pl.when(jnp.logical_and(step >= NSTEP - NJ, step < NSTEP))
                def _(): go(False)
        def wait(ref, sem):
            if dma: pltpu.make_async_copy(ref, ref, sem).wait()

        if dma:
            for b in range(NB):
                pltpu.make_async_copy(ax.at[b], xbuf.at[0, pl.ds(b * SQ, SQ)], xsem).start(priority=0)
                pltpu.make_async_copy(bx.at[b], xbuf.at[1, pl.ds(b * SQ, SQ)], xsem).start(priority=1)
            def wpro(qq, _):
                for n, c in enumerate(weight_copies(0, qq)): c.start(priority=n % 2)
            lax.fori_loop(0, 4, wpro, None)
        acc[...] = jnp.zeros(acc.shape, acc.dtype)
        if dma:
            def pro(s, _): issue(s, 0, 176, static_step=True)
            lax.fori_loop(0, 2, pro, None)
        wait(xbuf, xsem)

        def ld(ref32, *idx): return pltpu.bitcast(ref32[idx], jnp.bfloat16)
        def qk(q, k): return lax.dot_general(q, k, (((1,), (1,)), ((), ())), preferred_element_type=jnp.float32)
        def soft(s):
            m = jnp.max(s, axis=-1, keepdims=True)
            p = jnp.exp2(s - m)
            l = jnp.sum(p, axis=-1, keepdims=True)
            return p.astype(jnp.bfloat16), 1.0 / l
        def pv(p, r, v): return (jnp.dot(p, v, preferred_element_type=jnp.float32) * r).astype(jnp.bfloat16)
        def qproj(t, g, r0):
            q = jnp.dot(xbuf[t, pl.ds(r0, ROWS), :], w[g, t], preferred_element_type=jnp.float32)
            return (q * QSCALE).astype(jnp.bfloat16)
        def oproj(t, g, r0, o):
            acc[t, pl.ds(r0, ROWS), :] += jnp.dot(o, w[g, 2 + t], preferred_element_type=jnp.float32)
        def blk(x, i, hh): return x[i * SQ:(i + 1) * SQ, hh * DH:(hh + 1) * DH]

        def step_fn(s, _):
            g = s // NJ; j = s % NJ; slot = s % NSLOT
            r0 = pl.multiple_of(j * ROWS, ROWS)
            @pl.when(j == 0)
            def _(): wait(w.at[g], wsem.at[g])
            issue(s + 2, cuts[0], cuts[1])
            if compute: q = qproj(0, g, r0)
            issue(s + 2, cuts[1], cuts[2])
            wait(kva.at[slot], asem.at[slot])
            if compute:
                qs = [jnp.concatenate([blk(q, i, hh) for hh in range(4)], axis=0) for i in range(GB)]
                ss = [qk(qs[i], ld(kva32, slot, 0, i)) for i in range(GB)]
                ps = [soft(x) for x in ss]
                os_ = [pv(*ps[i], ld(kva32, slot, 1, i)) for i in range(GB)]
                o = jnp.concatenate([jnp.concatenate([os_[i][hh * SQ:(hh + 1) * SQ] for hh in range(4)], axis=1) for i in range(GB)], axis=0)
            issue(s + 2, cuts[2], cuts[3])
            if compute: oproj(0, g, r0, o)
            issue(s + 2, cuts[3], cuts[4])
            if compute: q = qproj(1, g, r0)
            issue(s + 2, cuts[4], cuts[5])
            wait(kvb.at[slot], bsem.at[slot])
            if compute:
                U = [(i, hh) for i in range(GB) for hh in range(4)]
                ss = [qk(blk(q, i, hh), ld(kvb32, slot, 0, i, hh)) for i, hh in U]
                ps = [soft(x) for x in ss]
                os_ = [pv(*ps[n], ld(kvb32, slot, 1, i, hh)) for n, (i, hh) in enumerate(U)]
                o = jnp.concatenate([jnp.concatenate(os_[4 * i:4 * i + 4], axis=1) for i in range(GB)], axis=0)
            issue(s + 2, cuts[5], cuts[6])
            if compute: oproj(1, g, r0, o)
            @pl.when(g == NG - 1)
            def _():
                for t in range(2):
                    ostage[pl.ds(r0, ROWS), t * D:(t + 1) * D] = acc[t, pl.ds(r0, ROWS), :].astype(jnp.bfloat16)
                pltpu.make_async_copy(ostage.at[pl.ds(r0, ROWS)], out.at[pl.ds(r0, ROWS)], osem).start()
        lax.fori_loop(0, NSTEP, step_fn, None)
        pltpu.make_async_copy(ostage, out, osem).wait()

    def fn(ax, ak, av, awq, awo, bx, bk, bv, bwq, bwo):
        bf = jnp.bfloat16
        out = pl.pallas_call(kernel,
            out_shape=jax.ShapeDtypeStruct((NB * SQ, 2 * D), bf),
            in_specs=[pl.BlockSpec(memory_space=pltpu.HBM)] * 10,
            out_specs=pl.BlockSpec(memory_space=pltpu.HBM),
            scratch_shapes=[
                pltpu.VMEM((2, NB * SQ, D), bf), pltpu.VMEM((NG, 4, 512, 512), bf),
                pltpu.VMEM((NSLOT, 2, GB, SK, DH), bf), pltpu.VMEM((NSLOT, 2, GB, 4, SK, DH), bf),
                pltpu.VMEM((2, NB * SQ, D), jnp.float32), pltpu.VMEM((NB * SQ, 2 * D), bf),
                pltpu.SemaphoreType.DMA((NSLOT,)), pltpu.SemaphoreType.DMA((NSLOT,)), pltpu.SemaphoreType.DMA((NG,)),
                pltpu.SemaphoreType.DMA(()), pltpu.SemaphoreType.DMA(()),
            ],
            compiler_params=pltpu.CompilerParams(vmem_limit_bytes=100 * 1024 * 1024, flags=flags, disable_bounds_checks=True),
        )(ax, ak, av, awq, awo, bx, bk, bv, bwq, bwo)
        return out.reshape(NB, SQ, 2 * D)
    return fn


_fn = make(order="h4")


@jax.jit
def pallas_concat_heads__gqa_block_cached__mha_block_cached__near_ridge_kernel(
    A_x, A_k_cache, A_v_cache, A_wq, A_wo, B_x, B_k_cache, B_v_cache, B_wq, B_wo,
):
    return _fn(A_x, A_k_cache, A_v_cache, A_wq, A_wo, B_x, B_k_cache, B_v_cache, B_wq, B_wo)
```

```python
import jax
import jax.numpy as jnp
import numpy as np
from jax import lax
import jax.experimental.pallas as pl
import jax.experimental.pallas.tpu as pltpu

NB, SQ, D, SK, DH = 16, 32, 512, 512, 128
NH = 32
GH = 4
GB = 4
NG = NH // GH
NJ = NB // GB
NSTEP = NG * NJ
ROWS = GB * SQ
GW = GH * DH
PIECE = 128
NP = SK // PIECE
A_ROWS = NP
SET_ROWS = NP + GH * NP
MARKS = (18, 20, 23, 26, 30, 34, 38)
QSCALE = float(DH ** -0.5 * np.log2(np.e))


def _batch(j, i):
    return j + i * NJ


def _kernel(ax, ak, av, awq, awo, bx, bk, bv, bwq, bwo, out,
            xbuf, wq, wo, kva, kvb, acc, stage, asem, bsem, wsem, osem):
    def fetch_rows(step, lo, hi):
        g, j, slot = step // NJ, step % NJ, step % 2

        def a_row(c, _):
            r = pl.ds(pl.multiple_of(c * PIECE, PIECE), PIECE)
            for i in range(GB):
                for t, src in enumerate((ak, av)):
                    pltpu.make_async_copy(
                        src.at[_batch(j, i), g, r], kva.at[slot, t, i, r], asem.at[slot]
                    ).start(priority=t)

        def b_row(n, _):
            h = n // NP
            r = pl.ds(pl.multiple_of((n % NP) * PIECE, PIECE), PIECE)
            for i in range(GB):
                for t, src in enumerate((bk, bv)):
                    pltpu.make_async_copy(
                        src.at[_batch(j, i), g * GH + h, r], kvb.at[slot, t, i, h, r], bsem.at[slot, t]
                    ).start(priority=t)

        if lo < min(hi, A_ROWS):
            lax.fori_loop(lo, min(hi, A_ROWS), a_row, None)
        if max(lo, A_ROWS) < hi:
            lax.fori_loop(max(lo, A_ROWS) - A_ROWS, hi - A_ROWS, b_row, None)

    def advance(step, mark):
        lo, hi = MARKS[mark], MARKS[mark + 1]
        if lo < min(hi, SET_ROWS):
            fetch_rows(step, lo, min(hi, SET_ROWS))
        if max(lo, SET_ROWS) < hi:
            @pl.when(step + 1 < NSTEP)
            def _():
                fetch_rows(step + 1, max(lo, SET_ROWS) - SET_ROWS, hi - SET_ROWS)

    def wait_filled(buf, sem):
        pltpu.make_async_copy(buf, buf, sem).wait()

    def write_group(j, half):
        for i in range(GB):
            pltpu.make_async_copy(
                stage.at[pl.ds((j * GB + i) * SQ + half * (SQ // 2), SQ // 2)],
                out.at[_batch(j, i), pl.ds(half * (SQ // 2), SQ // 2)],
                osem,
            ).start(priority=i % 2)

    def fetch_weights(n, _):
        for part in range(2):
            p = part * 64 + n
            rq = pl.ds(pl.multiple_of((p // 2) * 8, 8), 8)
            cq = pl.ds(pl.multiple_of((p % 2) * 2048, 2048), 2048)
            ro = pl.ds(pl.multiple_of(p * 32, 32), 32)
            for t, (sq, so) in enumerate(((awq, awo), (bwq, bwo))):
                pltpu.make_async_copy(sq.at[rq, cq], wq.at[t, rq, cq], wsem.at[0]).start(priority=0)
                pltpu.make_async_copy(so.at[ro], wo.at[t, ro], wsem.at[1]).start(priority=1)

    def fetch_x(j, _):
        for i in range(GB):
            r = pl.ds(pl.multiple_of((j * GB + i) * SQ, SQ), SQ)
            for t, src in enumerate((ax, bx)):
                pltpu.make_async_copy(src.at[_batch(j, i)], xbuf.at[t, r], wsem.at[2]).start(priority=t)

    lax.fori_loop(0, 64, fetch_weights, None)
    lax.fori_loop(0, NJ, fetch_x, None)
    acc[...] = jnp.zeros(acc.shape, acc.dtype)
    fetch_rows(0, 0, MARKS[0])
    wait_filled(wq, wsem.at[0])
    wait_filled(wo, wsem.at[1])
    wait_filled(xbuf, wsem.at[2])

    def scores(q, k):
        return lax.dot_general(q, k, (((1,), (1,)), ((), ())), preferred_element_type=jnp.float32)

    def softmax_parts(s):
        p = jnp.exp2(s - jnp.max(s, axis=-1, keepdims=True))
        return p.astype(jnp.bfloat16), 1.0 / jnp.sum(p, axis=-1, keepdims=True)

    def values(p, inv, v):
        return (jnp.dot(p, v, preferred_element_type=jnp.float32) * inv).astype(jnp.bfloat16)

    def head_block(x, i, h):
        return x[i * SQ:(i + 1) * SQ, h * DH:(h + 1) * DH]

    def run_step(s, _):
        g, j, slot = s // NJ, s % NJ, s % 2
        rows = pl.ds(pl.multiple_of(j * ROWS, ROWS), ROWS)
        cols = pl.ds(pl.multiple_of(g * GW, GW), GW)

        def project_q(t):
            q = jnp.dot(xbuf[t, rows, :], wq[t, :, cols], preferred_element_type=jnp.float32)
            return (q * QSCALE).astype(jnp.bfloat16)

        def project_out(t, o):
            y = acc[t, rows, :] + jnp.dot(o, wo[t, cols, :], preferred_element_type=jnp.float32)
            acc[t, rows, :] = y
            stage[rows, t * D:(t + 1) * D] = y.astype(jnp.bfloat16)

        advance(s, 0)
        q = project_q(0)
        advance(s, 1)
        wait_filled(kva.at[slot], asem.at[slot])
        qs = [jnp.concatenate([head_block(q, i, h) for h in range(GH)], axis=0) for i in range(GB)]
        ss = [scores(qs[i], kva[slot, 0, i]) for i in range(GB)]
        ps = [softmax_parts(x) for x in ss]
        os_ = [values(*ps[i], kva[slot, 1, i]) for i in range(GB)]
        o = jnp.concatenate(
            [jnp.concatenate([x[h * SQ:(h + 1) * SQ] for h in range(GH)], axis=1) for x in os_], axis=0)
        advance(s, 2)
        project_out(0, o)

        advance(s, 3)
        q = project_q(1)
        advance(s, 4)
        wait_filled(kvb.at[slot, 0], bsem.at[slot, 0])
        units = [(i, h) for i in range(GB) for h in range(GH)]
        ss = [scores(head_block(q, i, h), kvb[slot, 0, i, h]) for i, h in units]
        ps = [softmax_parts(x) for x in ss]
        advance(s, 5)

        @pl.when(s == NSTEP - 1)
        def _():
            for half in range(2):
                for jj in range(NJ - 1):
                    write_group(jj, half)

        wait_filled(kvb.at[slot, 1], bsem.at[slot, 1])
        os_ = [values(*ps[n], kvb[slot, 1, i, h]) for n, (i, h) in enumerate(units)]
        o = jnp.concatenate(
            [jnp.concatenate(os_[i * GH:(i + 1) * GH], axis=1) for i in range(GB)], axis=0)
        project_out(1, o)

    lax.fori_loop(0, NSTEP, run_step, None)
    for half in range(2):
        write_group(NJ - 1, half)
    wait_filled(stage, osem)


@jax.jit
def pallas_concat_heads__gqa_block_cached__mha_block_cached__near_ridge_kernel(
    A_x: jax.Array,
    A_k_cache: jax.Array,
    A_v_cache: jax.Array,
    A_wq: jax.Array,
    A_wo: jax.Array,
    B_x: jax.Array,
    B_k_cache: jax.Array,
    B_v_cache: jax.Array,
    B_wq: jax.Array,
    B_wo: jax.Array,
):
    assert A_x.shape == B_x.shape == (NB, SQ, D)
    assert A_k_cache.shape == A_v_cache.shape == (NB, NG, SK, DH)
    assert B_k_cache.shape == B_v_cache.shape == (NB, NH, SK, DH)
    assert A_wq.shape == B_wq.shape == (D, NH * DH)
    assert A_wo.shape == B_wo.shape == (NH * DH, D)
    bf16 = jnp.bfloat16
    return pl.pallas_call(
        _kernel,
        out_shape=jax.ShapeDtypeStruct((NB, SQ, 2 * D), bf16),
        in_specs=[pl.BlockSpec(memory_space=pltpu.HBM)] * 10,
        out_specs=pl.BlockSpec(memory_space=pltpu.HBM),
        scratch_shapes=[
            pltpu.VMEM((2, NB * SQ, D), bf16),
            pltpu.VMEM((2, D, NH * DH), bf16),
            pltpu.VMEM((2, NH * DH, D), bf16),
            pltpu.VMEM((2, 2, GB, SK, DH), bf16),
            pltpu.VMEM((2, 2, GB, GH, SK, DH), bf16),
            pltpu.VMEM((2, NB * SQ, D), jnp.float32),
            pltpu.VMEM((NB * SQ, 2 * D), bf16),
            pltpu.SemaphoreType.DMA((2,)),
            pltpu.SemaphoreType.DMA((2, 2)),
            pltpu.SemaphoreType.DMA((3,)),
            pltpu.SemaphoreType.DMA(()),
        ],
        compiler_params=pltpu.CompilerParams(
            vmem_limit_bytes=64 * 1024 * 1024,
            disable_bounds_checks=True,
        ),
    )(A_x, A_k_cache, A_v_cache, A_wq, A_wo, B_x, B_k_cache, B_v_cache, B_wq, B_wo)
```

```python
import jax
import jax.numpy as jnp
import numpy as np
from jax import lax
import jax.experimental.pallas as pl
import jax.experimental.pallas.tpu as pltpu

NB, SQ, D, SK, DH = 16, 32, 512, 512, 128
NH = 32
GH = 4
GB = 4
NG = NH // GH
NJ = NB // GB
NSTEP = NG * NJ
ROWS = GB * SQ
PIECE = 128
NP = SK // PIECE
A_ROWS = 2 * GB * NP // 8
B_ROWS = GB * GH * NP // 8
SET_ROWS = A_ROWS + 2 * B_ROWS
MARKS = (15, 20, 22, 24, 27, 33, 35)
QSCALE = float(DH ** -0.5 * np.log2(np.e))


def _batch(j, i):
    return j + i * NJ


def _b_head(g, h):
    return g + (h % 2) * 2 * NG + (h // 2) * NG


def _kernel(ax, ak, av, awq, awo, bx, bk, bv, bwq, bwo, out,
            xbuf, wq, wo, kva, kvb, acc, stage, asem, bsem, wsem, osem):
    def fetch_rows(step, lo, hi):
        g, j, slot = step // NJ, step % NJ, step % 2

        def a_row(c, _):
            r = pl.ds(pl.multiple_of(c * PIECE, PIECE), PIECE)
            for m in range(8):
                i, t = m % 2 + (m // 4) * 2, (m // 2) % 2
                pltpu.make_async_copy(
                    (ak, av)[t].at[_batch(j, i), g, r], kva.at[slot, t, i, r], asem.at[slot]
                ).start(priority=m % 2)

        def b_row(t):
            def row(n, _):
                r = pl.ds(pl.multiple_of((n // 2) * PIECE, PIECE), PIECE)
                for m in range(8):
                    i, h = (m % 2) * 2 + (m // 2) % 2, m // 4 + (n % 2) * 2
                    pltpu.make_async_copy(
                        (bk, bv)[t].at[_batch(j, i), _b_head(g, h), r],
                        kvb.at[slot, t, i, h, r],
                        bsem.at[slot, t],
                    ).start(priority=m % 2)
            return row

        first = 0
        for count, row in ((A_ROWS, a_row), (B_ROWS, b_row(0)), (B_ROWS, b_row(1))):
            a, b = max(lo - first, 0), min(hi - first, count)
            if a < b:
                lax.fori_loop(a, b, row, None)
            first += count

    def advance(step, mark):
        lo, hi = MARKS[mark], MARKS[mark + 1]
        if lo < min(hi, SET_ROWS):
            fetch_rows(step, lo, min(hi, SET_ROWS))
        if max(lo, SET_ROWS) < hi:
            @pl.when(step + 1 < NSTEP)
            def _():
                fetch_rows(step + 1, max(lo, SET_ROWS) - SET_ROWS, hi - SET_ROWS)

    def wait_filled(buf, sem):
        pltpu.make_async_copy(buf, buf, sem).wait()

    def write_group(j, half):
        for i in range(GB):
            pltpu.make_async_copy(
                stage.at[pl.ds((j * GB + i) * SQ + half * (SQ // 2), SQ // 2)],
                out.at[_batch(j, i), pl.ds(half * (SQ // 2), SQ // 2)],
                osem,
            ).start(priority=i % 2)

    def fetch_weights(n, _):
        for part in range(2):
            p = part * 64 + n
            rq = pl.ds(pl.multiple_of((p // 2) * 8, 8), 8)
            cq = pl.ds(pl.multiple_of((p % 2) * 2048, 2048), 2048)
            ro = pl.ds(pl.multiple_of(p * 32, 32), 32)
            for t, src in enumerate((awq, bwq)):
                pltpu.make_async_copy(src.at[rq, cq], wq.at[t, rq, cq], wsem.at[0]).start(priority=t)
            for t, src in enumerate((awo, bwo)):
                pltpu.make_async_copy(src.at[ro], wo.at[t, ro], wsem.at[1]).start(priority=t)

    def fetch_x(j, _):
        for i in range(GB):
            r = pl.ds(pl.multiple_of((j * GB + i) * SQ, SQ), SQ)
            for t, src in enumerate((ax, bx)):
                pltpu.make_async_copy(src.at[_batch(j, i)], xbuf.at[t, r], wsem.at[2]).start(priority=t)

    lax.fori_loop(0, NJ, fetch_x, None)
    lax.fori_loop(0, 64, fetch_weights, None)
    acc[...] = jnp.zeros(acc.shape, acc.dtype)
    fetch_rows(0, 0, MARKS[0])
    wait_filled(wq, wsem.at[0])
    wait_filled(wo, wsem.at[1])
    wait_filled(xbuf, wsem.at[2])

    def scores(q, k):
        return lax.dot_general(q, k, (((1,), (1,)), ((), ())), preferred_element_type=jnp.float32)

    def softmax_parts(s):
        p = jnp.exp2(s - jnp.max(s, axis=-1, keepdims=True))
        return p.astype(jnp.bfloat16), 1.0 / jnp.sum(p, axis=-1, keepdims=True)

    def values(p, inv, v):
        return (jnp.dot(p, v, preferred_element_type=jnp.float32) * inv).astype(jnp.bfloat16)

    def head_block(x, i, h):
        return x[i * SQ:(i + 1) * SQ, h * DH:(h + 1) * DH]

    def run_step(s, _):
        g, j, slot = s // NJ, s % NJ, s % 2
        rows = pl.ds(pl.multiple_of(j * ROWS, ROWS), ROWS)

        def head_cols(t):
            heads = [g * GH + h if t == 0 else _b_head(g, h) for h in range(GH)]
            return [pl.ds(pl.multiple_of(h * DH, DH), DH) for h in heads]

        def project_q(t):
            w = jnp.concatenate([wq[t, :, c] for c in head_cols(t)], axis=1)
            q = jnp.dot(xbuf[t, rows, :], w, preferred_element_type=jnp.float32)
            return (q * QSCALE).astype(jnp.bfloat16)

        def project_out(t, o):
            w = jnp.concatenate([wo[t, c, :] for c in head_cols(t)], axis=0)
            y = acc[t, rows, :] + jnp.dot(o, w, preferred_element_type=jnp.float32)
            acc[t, rows, :] = y
            stage[rows, t * D:(t + 1) * D] = y.astype(jnp.bfloat16)

        advance(s, 0)
        q = project_q(0)
        advance(s, 1)
        wait_filled(kva.at[slot], asem.at[slot])
        qs = [jnp.concatenate([head_block(q, i, h) for h in range(GH)], axis=0) for i in range(GB)]
        ss = [scores(qs[i], kva[slot, 0, i]) for i in range(GB)]
        ps = [softmax_parts(x) for x in ss]
        os_ = [values(*ps[i], kva[slot, 1, i]) for i in range(GB)]
        o = jnp.concatenate(
            [jnp.concatenate([x[h * SQ:(h + 1) * SQ] for h in range(GH)], axis=1) for x in os_], axis=0)
        advance(s, 2)
        project_out(0, o)

        advance(s, 3)
        q = project_q(1)
        advance(s, 4)
        wait_filled(kvb.at[slot, 0], bsem.at[slot, 0])
        units = [(i, h) for i in range(GB) for h in range(GH)]
        ss = [scores(head_block(q, i, h), kvb[slot, 0, i, h]) for i, h in units]
        ps = [softmax_parts(x) for x in ss]
        advance(s, 5)

        @pl.when(s == NSTEP - 1)
        def _():
            for half in range(2):
                for jj in range(NJ - 1):
                    write_group(jj, half)

        wait_filled(kvb.at[slot, 1], bsem.at[slot, 1])
        os_ = [values(*ps[n], kvb[slot, 1, i, h]) for n, (i, h) in enumerate(units)]
        o = jnp.concatenate(
            [jnp.concatenate(os_[i * GH:(i + 1) * GH], axis=1) for i in range(GB)], axis=0)
        project_out(1, o)

    lax.fori_loop(0, NSTEP, run_step, None)
    for half in range(2):
        write_group(NJ - 1, half)
    wait_filled(stage, osem)


@jax.jit
def pallas_concat_heads__gqa_block_cached__mha_block_cached__near_ridge_kernel(
    A_x: jax.Array,
    A_k_cache: jax.Array,
    A_v_cache: jax.Array,
    A_wq: jax.Array,
    A_wo: jax.Array,
    B_x: jax.Array,
    B_k_cache: jax.Array,
    B_v_cache: jax.Array,
    B_wq: jax.Array,
    B_wo: jax.Array,
):
    assert A_x.shape == B_x.shape == (NB, SQ, D)
    assert A_k_cache.shape == A_v_cache.shape == (NB, NG, SK, DH)
    assert B_k_cache.shape == B_v_cache.shape == (NB, NH, SK, DH)
    assert A_wq.shape == B_wq.shape == (D, NH * DH)
    assert A_wo.shape == B_wo.shape == (NH * DH, D)
    bf16 = jnp.bfloat16
    return pl.pallas_call(
        _kernel,
        out_shape=jax.ShapeDtypeStruct((NB, SQ, 2 * D), bf16),
        in_specs=[pl.BlockSpec(memory_space=pltpu.HBM)] * 10,
        out_specs=pl.BlockSpec(memory_space=pltpu.HBM),
        scratch_shapes=[
            pltpu.VMEM((2, NB * SQ, D), bf16),
            pltpu.VMEM((2, D, NH * DH), bf16),
            pltpu.VMEM((2, NH * DH, D), bf16),
            pltpu.VMEM((2, 2, GB, SK, DH), bf16),
            pltpu.VMEM((2, 2, GB, GH, SK, DH), bf16),
            pltpu.VMEM((2, NB * SQ, D), jnp.float32),
            pltpu.VMEM((NB * SQ, 2 * D), bf16),
            pltpu.SemaphoreType.DMA((2,)),
            pltpu.SemaphoreType.DMA((2, 2)),
            pltpu.SemaphoreType.DMA((3,)),
            pltpu.SemaphoreType.DMA(()),
        ],
        compiler_params=pltpu.CompilerParams(
            vmem_limit_bytes=64 * 1024 * 1024,
            disable_bounds_checks=True,
        ),
    )(A_x, A_k_cache, A_v_cache, A_wq, A_wo, B_x, B_k_cache, B_v_cache, B_wq, B_wo)
```

```python
import jax
import jax.numpy as jnp
import numpy as np
from jax import lax
import jax.experimental.pallas as pl
import jax.experimental.pallas.tpu as pltpu

NB, SQ, D, SK, DH = 16, 32, 512, 512, 128
NH = 32
GH = 4
GB = 4
NG = NH // GH
NJ = NB // GB
NSTEP = NG * NJ
ROWS = GB * SQ
PIECE = 128
NP = SK // PIECE
A_ROWS = 2 * GB * NP // 8
B_ROWS = GB * GH * NP // 8
SET_ROWS = A_ROWS + 2 * B_ROWS
MARKS = (15, 20, 22, 24, 27, 33, 35)
QSCALE = float(DH ** -0.5 * np.log2(np.e))


def _batch(j, i):
    return j + i * NJ


def _b_head(g, h):
    return g + (h % 2) * 2 * NG + (h // 2) * NG


def _kernel(ax, ak, av, awq, awo, bx, bk, bv, bwq, bwo, out,
            xbuf, wq, wo, kva, kvb, acc, stage, asem, bsem, wsem, osem):
    def fetch_rows(step, lo, hi):
        g, j, slot = step // NJ, step % NJ, step % 2

        def a_row(c, _):
            r = pl.ds(pl.multiple_of(c * PIECE, PIECE), PIECE)
            for m in range(8):
                i, t = m % 2 + (m // 4) * 2, (m // 2) % 2
                pltpu.make_async_copy(
                    (ak, av)[t].at[_batch(j, i), g, r], kva.at[slot, t, i, r], asem.at[slot]
                ).start(priority=m % 2)

        def b_row(t):
            def row(n, _):
                r = pl.ds(pl.multiple_of((n // 2) * PIECE, PIECE), PIECE)
                for m in range(8):
                    i, h = (m % 2) * 2 + (m // 2) % 2, m // 4 + (n % 2) * 2
                    pltpu.make_async_copy(
                        (bk, bv)[t].at[_batch(j, i), _b_head(g, h), r],
                        kvb.at[slot, t, i, h, r],
                        bsem.at[slot, t],
                    ).start(priority=m % 2)
            return row

        first = 0
        for count, row in ((A_ROWS, a_row), (B_ROWS, b_row(0)), (B_ROWS, b_row(1))):
            a, b = max(lo - first, 0), min(hi - first, count)
            if a < b:
                lax.fori_loop(a, b, row, None)
            first += count

    def advance(step, mark):
        lo, hi = MARKS[mark], MARKS[mark + 1]
        if lo < min(hi, SET_ROWS):
            fetch_rows(step, lo, min(hi, SET_ROWS))
        if max(lo, SET_ROWS) < hi:
            @pl.when(step + 1 < NSTEP)
            def _():
                fetch_rows(step + 1, max(lo, SET_ROWS) - SET_ROWS, hi - SET_ROWS)

    def wait_filled(buf, sem):
        pltpu.make_async_copy(buf, buf, sem).wait()

    def write_group(j, half):
        for i in range(GB):
            pltpu.make_async_copy(
                stage.at[pl.ds((j * GB + i) * SQ + half * (SQ // 2), SQ // 2)],
                out.at[_batch(j, i), pl.ds(half * (SQ // 2), SQ // 2)],
                osem,
            ).start(priority=i % 2)

    def fetch_weights(n, _):
        for part in range(2):
            p = part * 64 + n
            rq = pl.ds(pl.multiple_of((p // 2) * 8, 8), 8)
            cq = pl.ds(pl.multiple_of((p % 2) * 2048, 2048), 2048)
            ro = pl.ds(pl.multiple_of(p * 32, 32), 32)
            for t, src in enumerate((awq, bwq)):
                pltpu.make_async_copy(src.at[rq, cq], wq.at[t, rq, cq], wsem.at[0]).start(priority=t)
            for t, src in enumerate((awo, bwo)):
                pltpu.make_async_copy(src.at[ro], wo.at[t, ro], wsem.at[1]).start(priority=t)

    def fetch_x(j, _):
        for i in range(GB):
            r = pl.ds(pl.multiple_of((j * GB + i) * SQ, SQ), SQ)
            for t, src in enumerate((ax, bx)):
                pltpu.make_async_copy(src.at[_batch(j, i)], xbuf.at[t, r], wsem.at[2]).start(priority=1)

    lax.fori_loop(0, NJ, fetch_x, None)
    lax.fori_loop(0, 64, fetch_weights, None)
    acc[...] = jnp.zeros(acc.shape, acc.dtype)
    fetch_rows(0, 0, MARKS[0])
    wait_filled(wq, wsem.at[0])
    wait_filled(wo, wsem.at[1])
    wait_filled(xbuf, wsem.at[2])

    def scores(q, k):
        return lax.dot_general(q, k, (((1,), (1,)), ((), ())), preferred_element_type=jnp.float32)

    def softmax_parts(s):
        p = jnp.exp2(s - jnp.max(s, axis=-1, keepdims=True))
        return p.astype(jnp.bfloat16), 1.0 / jnp.sum(p, axis=-1, keepdims=True)

    def values(p, inv, v):
        return (jnp.dot(p, v, preferred_element_type=jnp.float32) * inv).astype(jnp.bfloat16)

    def head_block(x, i, h):
        return x[i * SQ:(i + 1) * SQ, h * DH:(h + 1) * DH]

    def run_step(s, _):
        g, j, slot = s // NJ, s % NJ, s % 2
        rows = pl.ds(pl.multiple_of(j * ROWS, ROWS), ROWS)

        def head_cols(t):
            heads = [g * GH + h if t == 0 else _b_head(g, h) for h in range(GH)]
            return [pl.ds(pl.multiple_of(h * DH, DH), DH) for h in heads]

        def project_q(t):
            w = jnp.concatenate([wq[t, :, c] for c in head_cols(t)], axis=1)
            q = jnp.dot(xbuf[t, rows, :], w, preferred_element_type=jnp.float32)
            return (q * QSCALE).astype(jnp.bfloat16)

        def project_out(t, o):
            w = jnp.concatenate([wo[t, c, :] for c in head_cols(t)], axis=0)
            y = acc[t, rows, :] + jnp.dot(o, w, preferred_element_type=jnp.float32)
            acc[t, rows, :] = y
            stage[rows, t * D:(t + 1) * D] = y.astype(jnp.bfloat16)

        advance(s, 0)
        q = project_q(0)
        advance(s, 1)
        wait_filled(kva.at[slot], asem.at[slot])
        qs = [jnp.concatenate([head_block(q, i, h) for h in range(GH)], axis=0) for i in range(GB)]
        ss = [scores(qs[i], kva[slot, 0, i]) for i in range(GB)]
        ps = [softmax_parts(x) for x in ss]
        os_ = [values(*ps[i], kva[slot, 1, i]) for i in range(GB)]
        o = jnp.concatenate(
            [jnp.concatenate([x[h * SQ:(h + 1) * SQ] for h in range(GH)], axis=1) for x in os_], axis=0)
        advance(s, 2)
        project_out(0, o)

        advance(s, 3)
        q = project_q(1)
        advance(s, 4)
        wait_filled(kvb.at[slot, 0], bsem.at[slot, 0])
        units = [(i, h) for i in range(GB) for h in range(GH)]
        ss = [scores(head_block(q, i, h), kvb[slot, 0, i, h]) for i, h in units]
        ps = [softmax_parts(x) for x in ss]
        advance(s, 5)

        @pl.when(s == NSTEP - 1)
        def _():
            for half in range(2):
                for jj in range(NJ - 1):
                    write_group(jj, half)

        wait_filled(kvb.at[slot, 1], bsem.at[slot, 1])
        os_ = [values(*ps[n], kvb[slot, 1, i, h]) for n, (i, h) in enumerate(units)]
        o = jnp.concatenate(
            [jnp.concatenate(os_[i * GH:(i + 1) * GH], axis=1) for i in range(GB)], axis=0)
        project_out(1, o)

    lax.fori_loop(0, NSTEP, run_step, None)
    for half in range(2):
        write_group(NJ - 1, half)
    wait_filled(stage, osem)


@jax.jit
def pallas_concat_heads__gqa_block_cached__mha_block_cached__near_ridge_kernel(
    A_x: jax.Array,
    A_k_cache: jax.Array,
    A_v_cache: jax.Array,
    A_wq: jax.Array,
    A_wo: jax.Array,
    B_x: jax.Array,
    B_k_cache: jax.Array,
    B_v_cache: jax.Array,
    B_wq: jax.Array,
    B_wo: jax.Array,
):
    assert A_x.shape == B_x.shape == (NB, SQ, D)
    assert A_k_cache.shape == A_v_cache.shape == (NB, NG, SK, DH)
    assert B_k_cache.shape == B_v_cache.shape == (NB, NH, SK, DH)
    assert A_wq.shape == B_wq.shape == (D, NH * DH)
    assert A_wo.shape == B_wo.shape == (NH * DH, D)
    bf16 = jnp.bfloat16
    return pl.pallas_call(
        _kernel,
        out_shape=jax.ShapeDtypeStruct((NB, SQ, 2 * D), bf16),
        in_specs=[pl.BlockSpec(memory_space=pltpu.HBM)] * 10,
        out_specs=pl.BlockSpec(memory_space=pltpu.HBM),
        scratch_shapes=[
            pltpu.VMEM((2, NB * SQ, D), bf16),
            pltpu.VMEM((2, D, NH * DH), bf16),
            pltpu.VMEM((2, NH * DH, D), bf16),
            pltpu.VMEM((2, 2, GB, SK, DH), bf16),
            pltpu.VMEM((2, 2, GB, GH, SK, DH), bf16),
            pltpu.VMEM((2, NB * SQ, D), jnp.float32),
            pltpu.VMEM((NB * SQ, 2 * D), bf16),
            pltpu.SemaphoreType.DMA((2,)),
            pltpu.SemaphoreType.DMA((2, 2)),
            pltpu.SemaphoreType.DMA((3,)),
            pltpu.SemaphoreType.DMA(()),
        ],
        compiler_params=pltpu.CompilerParams(vmem_limit_bytes=64 * 1024 * 1024),
    )(A_x, A_k_cache, A_v_cache, A_wq, A_wo, B_x, B_k_cache, B_v_cache, B_wq, B_wo)
```

```python
import jax
import jax.numpy as jnp
import numpy as np
from jax import lax
import jax.experimental.pallas as pl
import jax.experimental.pallas.tpu as pltpu

NB, SQ, D, SK, DH = 16, 32, 512, 512, 128
NH = 32
GH = 4
GB = 4
NG = NH // GH
NJ = NB // GB
NSTEP = NG * NJ
ROWS = GB * SQ
PIECE = 128
NP = SK // PIECE
A_ROWS = 2 * GB * NP // 8
B_ROWS = GB * GH * NP // 8
SET_ROWS = A_ROWS + 2 * B_ROWS
MARKS = (15, 20, 22, 24, 27, 33, 35)
QSCALE = float(DH ** -0.5 * np.log2(np.e))


def _divmod(x, n):
    return x >> (n.bit_length() - 1), x & (n - 1)


def _batch(j, i):
    return j + i * NJ


def _b_head(g, pair, odd):
    return g + pair * NG + odd * 2 * NG


def _kernel(ax, ak, av, awq, awo, bx, bk, bv, bwq, bwo, out,
            xbuf, wq, wo, kva, kvb, acc, stage, asem, bsem, wsem, osem):
    def fetch_rows(step, lo, hi):
        (g, j), slot = _divmod(step, NJ), step & 1

        def a_row(c, _):
            r = pl.ds(pl.multiple_of(c * PIECE, PIECE), PIECE)
            for m in range(8):
                i, t = m % 2 + (m // 4) * 2, (m // 2) % 2
                pltpu.make_async_copy(
                    (ak, av)[t].at[_batch(j, i), g, r], kva.at[slot, t, i, r], asem.at[slot]
                ).start(priority=m % 2)

        def b_row(t):
            def row(n, _):
                c, pair = _divmod(n, 2)
                r = pl.ds(pl.multiple_of(c * PIECE, PIECE), PIECE)
                for m in range(8):
                    i, odd = (m % 2) * 2 + (m // 2) % 2, m // 4
                    pltpu.make_async_copy(
                        (bk, bv)[t].at[_batch(j, i), _b_head(g, pair, odd), r],
                        kvb.at[slot, t, i, 2 * pair + odd, r],
                        bsem.at[slot, t],
                    ).start(priority=m % 2)
            return row

        first = 0
        for count, row in ((A_ROWS, a_row), (B_ROWS, b_row(0)), (B_ROWS, b_row(1))):
            a, b = max(lo - first, 0), min(hi - first, count)
            if a < b:
                lax.fori_loop(a, b, row, None)
            first += count

    def advance(step, mark):
        lo, hi = MARKS[mark], MARKS[mark + 1]
        if lo < min(hi, SET_ROWS):
            fetch_rows(step, lo, min(hi, SET_ROWS))
        if max(lo, SET_ROWS) < hi:
            @pl.when(step + 1 < NSTEP)
            def _():
                fetch_rows(step + 1, max(lo, SET_ROWS) - SET_ROWS, hi - SET_ROWS)

    def wait_filled(buf, sem):
        pltpu.make_async_copy(buf, buf, sem).wait()

    def write_group(j, half):
        for i in range(GB):
            pltpu.make_async_copy(
                stage.at[pl.ds((j * GB + i) * SQ + half * (SQ // 2), SQ // 2)],
                out.at[_batch(j, i), pl.ds(half * (SQ // 2), SQ // 2)],
                osem,
            ).start(priority=i % 2)

    def fetch_weights(n, _):
        for part in range(2):
            p = part * 64 + n
            band, side = _divmod(p, 2)
            rq = pl.ds(pl.multiple_of(band * 8, 8), 8)
            cq = pl.ds(pl.multiple_of(side * 2048, 2048), 2048)
            ro = pl.ds(pl.multiple_of(p * 32, 32), 32)
            for t, src in enumerate((awq, bwq)):
                pltpu.make_async_copy(src.at[rq, cq], wq.at[t, rq, cq], wsem.at[0]).start(priority=t)
            for t, src in enumerate((awo, bwo)):
                pltpu.make_async_copy(src.at[ro], wo.at[t, ro], wsem.at[1]).start(priority=t)

    def fetch_x(j, _):
        for i in range(GB):
            r = pl.ds(pl.multiple_of((j * GB + i) * SQ, SQ), SQ)
            for t, src in enumerate((ax, bx)):
                pltpu.make_async_copy(src.at[_batch(j, i)], xbuf.at[t, r], wsem.at[2]).start(priority=1)

    lax.fori_loop(0, NJ, fetch_x, None)
    lax.fori_loop(0, 64, fetch_weights, None)
    acc[...] = jnp.zeros(acc.shape, acc.dtype)
    fetch_rows(0, 0, MARKS[0])
    wait_filled(wq, wsem.at[0])
    wait_filled(wo, wsem.at[1])
    wait_filled(xbuf, wsem.at[2])

    def scores(q, k):
        return lax.dot_general(q, k, (((1,), (1,)), ((), ())), preferred_element_type=jnp.float32)

    def softmax_parts(s):
        p = jnp.exp2(s - jnp.max(s, axis=-1, keepdims=True))
        return p.astype(jnp.bfloat16), 1.0 / jnp.sum(p, axis=-1, keepdims=True)

    def values(p, inv, v):
        return (jnp.dot(p, v, preferred_element_type=jnp.float32) * inv).astype(jnp.bfloat16)

    def head_block(x, i, h):
        return x[i * SQ:(i + 1) * SQ, h * DH:(h + 1) * DH]

    def run_step(s, _):
        (g, j), slot = _divmod(s, NJ), s & 1
        rows = pl.ds(pl.multiple_of(j * ROWS, ROWS), ROWS)

        def head_cols(t):
            heads = [g * GH + h if t == 0 else _b_head(g, h // 2, h % 2) for h in range(GH)]
            return [pl.ds(pl.multiple_of(h * DH, DH), DH) for h in heads]

        def project_q(t):
            w = jnp.concatenate([wq[t, :, c] for c in head_cols(t)], axis=1)
            q = jnp.dot(xbuf[t, rows, :], w, preferred_element_type=jnp.float32)
            return (q * QSCALE).astype(jnp.bfloat16)

        def project_out(t, o):
            w = jnp.concatenate([wo[t, c, :] for c in head_cols(t)], axis=0)
            y = acc[t, rows, :] + jnp.dot(o, w, preferred_element_type=jnp.float32)
            acc[t, rows, :] = y
            stage[rows, t * D:(t + 1) * D] = y.astype(jnp.bfloat16)

        advance(s, 0)
        q = project_q(0)
        advance(s, 1)
        wait_filled(kva.at[slot], asem.at[slot])
        qs = [jnp.concatenate([head_block(q, i, h) for h in range(GH)], axis=0) for i in range(GB)]
        ss = [scores(qs[i], kva[slot, 0, i]) for i in range(GB)]
        ps = [softmax_parts(x) for x in ss]
        os_ = [values(*ps[i], kva[slot, 1, i]) for i in range(GB)]
        o = jnp.concatenate(
            [jnp.concatenate([x[h * SQ:(h + 1) * SQ] for h in range(GH)], axis=1) for x in os_], axis=0)
        advance(s, 2)
        project_out(0, o)

        advance(s, 3)
        q = project_q(1)
        advance(s, 4)
        wait_filled(kvb.at[slot, 0], bsem.at[slot, 0])
        units = [(i, h) for i in range(GB) for h in range(GH)]
        ss = [scores(head_block(q, i, h), kvb[slot, 0, i, h]) for i, h in units]
        ps = [softmax_parts(x) for x in ss]
        advance(s, 5)

        @pl.when(s == NSTEP - 1)
        def _():
            for half in range(2):
                for jj in range(NJ - 1):
                    write_group(jj, half)

        wait_filled(kvb.at[slot, 1], bsem.at[slot, 1])
        os_ = [values(*ps[n], kvb[slot, 1, i, h]) for n, (i, h) in enumerate(units)]
        o = jnp.concatenate(
            [jnp.concatenate(os_[i * GH:(i + 1) * GH], axis=1) for i in range(GB)], axis=0)
        project_out(1, o)

    lax.fori_loop(0, NSTEP, run_step, None)
    for half in range(2):
        write_group(NJ - 1, half)
    wait_filled(stage, osem)


@jax.jit
def pallas_concat_heads__gqa_block_cached__mha_block_cached__near_ridge_kernel(
    A_x: jax.Array,
    A_k_cache: jax.Array,
    A_v_cache: jax.Array,
    A_wq: jax.Array,
    A_wo: jax.Array,
    B_x: jax.Array,
    B_k_cache: jax.Array,
    B_v_cache: jax.Array,
    B_wq: jax.Array,
    B_wo: jax.Array,
):
    assert A_x.shape == B_x.shape == (NB, SQ, D)
    assert A_k_cache.shape == A_v_cache.shape == (NB, NG, SK, DH)
    assert B_k_cache.shape == B_v_cache.shape == (NB, NH, SK, DH)
    assert A_wq.shape == B_wq.shape == (D, NH * DH)
    assert A_wo.shape == B_wo.shape == (NH * DH, D)
    bf16 = jnp.bfloat16
    return pl.pallas_call(
        _kernel,
        out_shape=jax.ShapeDtypeStruct((NB, SQ, 2 * D), bf16),
        in_specs=[pl.BlockSpec(memory_space=pltpu.HBM)] * 10,
        out_specs=pl.BlockSpec(memory_space=pltpu.HBM),
        scratch_shapes=[
            pltpu.VMEM((2, NB * SQ, D), bf16),
            pltpu.VMEM((2, D, NH * DH), bf16),
            pltpu.VMEM((2, NH * DH, D), bf16),
            pltpu.VMEM((2, 2, GB, SK, DH), bf16),
            pltpu.VMEM((2, 2, GB, GH, SK, DH), bf16),
            pltpu.VMEM((2, NB * SQ, D), jnp.float32),
            pltpu.VMEM((NB * SQ, 2 * D), bf16),
            pltpu.SemaphoreType.DMA((2,)),
            pltpu.SemaphoreType.DMA((2, 2)),
            pltpu.SemaphoreType.DMA((3,)),
            pltpu.SemaphoreType.DMA(()),
        ],
        compiler_params=pltpu.CompilerParams(vmem_limit_bytes=64 * 1024 * 1024),
    )(A_x, A_k_cache, A_v_cache, A_wq, A_wo, B_x, B_k_cache, B_v_cache, B_wq, B_wo)
```

```python
import functools

import jax
import jax.numpy as jnp
import numpy as np
from jax import lax
import jax.experimental.pallas as pl
import jax.experimental.pallas.tpu as pltpu

NB, SQ, D, SK, DH = 16, 32, 512, 512, 128
NH = 32
GH = 4
GB = 4
NG = NH // GH
NJ = NB // GB
NSTEP = NG * NJ
ROWS = GB * SQ
PIECE = 128
NP = SK // PIECE
A_ROWS = 2 * GB * NP // 8
B_ROWS = GB * GH * NP // 8
SET_ROWS = A_ROWS + 2 * B_ROWS
MARKS = (15, 18, 21, 24, 27, 33, 35)
QSCALE = float(DH ** -0.5 * np.log2(np.e))


def _divmod(x, n):
    return x >> (n.bit_length() - 1), x & (n - 1)


def _batch(j, i):
    return j + i * NJ


def _b_head(g, pair, odd):
    return g + pair * NG + odd * 2 * NG


def _wait_filled(buf, sem):
    pltpu.make_async_copy(buf, buf, sem).wait()


def _kernel(*refs):
    out, osem = refs[10], refs[-1]
    pl.run_scoped(
        functools.partial(_run, *refs),
        pltpu.SemaphoreType.DMA((2,)),
        pltpu.SemaphoreType.DMA((2, 2)),
        pltpu.SemaphoreType.DMA((3,)),
    )
    _wait_filled(out, osem)


def _run(ax, ak, av, awq, awo, bx, bk, bv, bwq, bwo, out,
         xbuf, wq, wo, kva, kvb, acc, stage, osem, asem, bsem, wsem):
    def fetch_rows(step, lo, hi):
        (g, j), slot = _divmod(step, NJ), step & 1

        def a_row(c, _):
            r = pl.ds(pl.multiple_of(c * PIECE, PIECE), PIECE)
            for m in range(8):
                i, t = m % 2 + (m // 4) * 2, (m // 2) % 2
                pltpu.make_async_copy(
                    (ak, av)[t].at[_batch(j, i), g, r], kva.at[slot, t, i, r], asem.at[slot]
                ).start(priority=m % 2)

        def b_row(t):
            def row(n, _):
                c, pair = _divmod(n, 2)
                r = pl.ds(pl.multiple_of(c * PIECE, PIECE), PIECE)
                for m in range(8):
                    i, odd = (m % 2) * 2 + (m // 2) % 2, m // 4
                    pltpu.make_async_copy(
                        (bk, bv)[t].at[_batch(j, i), _b_head(g, pair, odd), r],
                        kvb.at[slot, t, i, 2 * pair + odd, r],
                        bsem.at[slot, t],
                    ).start(priority=m % 2)
            return row

        first = 0
        for count, row in ((A_ROWS, a_row), (B_ROWS, b_row(0)), (B_ROWS, b_row(1))):
            a, b = max(lo - first, 0), min(hi - first, count)
            if a < b:
                lax.fori_loop(a, b, row, None)
            first += count

    def advance(step, mark):
        lo, hi = MARKS[mark], MARKS[mark + 1]
        if lo < min(hi, SET_ROWS):
            fetch_rows(step, lo, min(hi, SET_ROWS))
        if max(lo, SET_ROWS) < hi:
            @pl.when(step + 1 < NSTEP)
            def _():
                fetch_rows(step + 1, max(lo, SET_ROWS) - SET_ROWS, hi - SET_ROWS)

    def write_group(j, half):
        for i in range(GB):
            pltpu.make_async_copy(
                stage.at[pl.ds((j * GB + i) * SQ + half * (SQ // 2), SQ // 2)],
                out.at[_batch(j, i), pl.ds(half * (SQ // 2), SQ // 2)],
                osem,
            ).start(priority=i % 2)

    def fetch_weights(n, _):
        for part in range(2):
            p = part * 64 + n
            band, side = _divmod(p, 2)
            rq = pl.ds(pl.multiple_of(band * 8, 8), 8)
            cq = pl.ds(pl.multiple_of(side * 2048, 2048), 2048)
            ro = pl.ds(pl.multiple_of(p * 32, 32), 32)
            for t, src in enumerate((awq, bwq)):
                pltpu.make_async_copy(src.at[rq, cq], wq.at[t, rq, cq], wsem.at[0]).start(priority=t)
            for t, src in enumerate((awo, bwo)):
                pltpu.make_async_copy(src.at[ro], wo.at[t, ro], wsem.at[1]).start(priority=t)

    def fetch_x(j, _):
        for i in range(GB):
            r = pl.ds(pl.multiple_of((j * GB + i) * SQ, SQ), SQ)
            for t, src in enumerate((ax, bx)):
                pltpu.make_async_copy(src.at[_batch(j, i)], xbuf.at[t, r], wsem.at[2]).start(priority=1)

    lax.fori_loop(0, NJ, fetch_x, None)
    lax.fori_loop(0, 64, fetch_weights, None)
    acc[...] = jnp.zeros(acc.shape, acc.dtype)
    fetch_rows(0, 0, MARKS[0])
    _wait_filled(wq, wsem.at[0])
    _wait_filled(wo, wsem.at[1])
    _wait_filled(xbuf, wsem.at[2])

    def scores(q, k):
        return lax.dot_general(q, k, (((1,), (1,)), ((), ())), preferred_element_type=jnp.float32)

    def softmax_parts(s):
        p = jnp.exp2(s - jnp.max(s, axis=-1, keepdims=True))
        return p.astype(jnp.bfloat16), 1.0 / jnp.sum(p, axis=-1, keepdims=True)

    def values(p, inv, v):
        return (jnp.dot(p, v, preferred_element_type=jnp.float32) * inv).astype(jnp.bfloat16)

    def head_block(x, i, h):
        return x[i * SQ:(i + 1) * SQ, h * DH:(h + 1) * DH]

    def run_step(s, _):
        (g, j), slot = _divmod(s, NJ), s & 1
        rows = pl.ds(pl.multiple_of(j * ROWS, ROWS), ROWS)

        def head_cols(t):
            heads = [g * GH + h if t == 0 else _b_head(g, h // 2, h % 2) for h in range(GH)]
            return [pl.ds(pl.multiple_of(h * DH, DH), DH) for h in heads]

        def project_q(t):
            w = jnp.concatenate([wq[t, :, c] for c in head_cols(t)], axis=1)
            q = jnp.dot(xbuf[t, rows, :], w, preferred_element_type=jnp.float32)
            return (q * QSCALE).astype(jnp.bfloat16)

        def project_out(t, o):
            w = jnp.concatenate([wo[t, c, :] for c in head_cols(t)], axis=0)
            y = acc[t, rows, :] + jnp.dot(o, w, preferred_element_type=jnp.float32)
            acc[t, rows, :] = y
            stage[rows, t * D:(t + 1) * D] = y.astype(jnp.bfloat16)

        advance(s, 0)
        q = project_q(0)
        advance(s, 1)
        _wait_filled(kva.at[slot], asem.at[slot])
        qs = [jnp.concatenate([head_block(q, i, h) for h in range(GH)], axis=0) for i in range(GB)]
        ss = [scores(qs[i], kva[slot, 0, i]) for i in range(GB)]
        ps = [softmax_parts(x) for x in ss]
        os_ = [values(*ps[i], kva[slot, 1, i]) for i in range(GB)]
        o = jnp.concatenate(
            [jnp.concatenate([x[h * SQ:(h + 1) * SQ] for h in range(GH)], axis=1) for x in os_], axis=0)
        advance(s, 2)
        project_out(0, o)

        advance(s, 3)
        q = project_q(1)
        advance(s, 4)
        _wait_filled(kvb.at[slot, 0], bsem.at[slot, 0])
        units = [(i, h) for i in range(GB) for h in range(GH)]
        ss = [scores(head_block(q, i, h), kvb[slot, 0, i, h]) for i, h in units]
        ps = [softmax_parts(x) for x in ss]
        advance(s, 5)

        @pl.when(s == NSTEP - 1)
        def _():
            for half in range(2):
                for jj in range(NJ - 1):
                    write_group(jj, half)

        _wait_filled(kvb.at[slot, 1], bsem.at[slot, 1])
        os_ = [values(*ps[n], kvb[slot, 1, i, h]) for n, (i, h) in enumerate(units)]
        o = jnp.concatenate(
            [jnp.concatenate(os_[i * GH:(i + 1) * GH], axis=1) for i in range(GB)], axis=0)
        project_out(1, o)

    lax.fori_loop(0, NSTEP, run_step, None)
    for half in range(2):
        write_group(NJ - 1, half)


@jax.jit
def pallas_concat_heads__gqa_block_cached__mha_block_cached__near_ridge_kernel(
    A_x: jax.Array,
    A_k_cache: jax.Array,
    A_v_cache: jax.Array,
    A_wq: jax.Array,
    A_wo: jax.Array,
    B_x: jax.Array,
    B_k_cache: jax.Array,
    B_v_cache: jax.Array,
    B_wq: jax.Array,
    B_wo: jax.Array,
):
    assert A_x.shape == B_x.shape == (NB, SQ, D)
    assert A_k_cache.shape == A_v_cache.shape == (NB, NG, SK, DH)
    assert B_k_cache.shape == B_v_cache.shape == (NB, NH, SK, DH)
    assert A_wq.shape == B_wq.shape == (D, NH * DH)
    assert A_wo.shape == B_wo.shape == (NH * DH, D)
    bf16 = jnp.bfloat16
    return pl.pallas_call(
        _kernel,
        out_shape=jax.ShapeDtypeStruct((NB, SQ, 2 * D), bf16),
        in_specs=[pl.BlockSpec(memory_space=pltpu.HBM)] * 10,
        out_specs=pl.BlockSpec(memory_space=pltpu.HBM),
        scratch_shapes=[
            pltpu.VMEM((2, NB * SQ, D), bf16),
            pltpu.VMEM((2, D, NH * DH), bf16),
            pltpu.VMEM((2, NH * DH, D), bf16),
            pltpu.VMEM((2, 2, GB, SK, DH), bf16),
            pltpu.VMEM((2, 2, GB, GH, SK, DH), bf16),
            pltpu.VMEM((2, NB * SQ, D), jnp.float32),
            pltpu.VMEM((NB * SQ, 2 * D), bf16),
            pltpu.SemaphoreType.DMA(()),
        ],
        compiler_params=pltpu.CompilerParams(vmem_limit_bytes=64 * 1024 * 1024),
    )(A_x, A_k_cache, A_v_cache, A_wq, A_wo, B_x, B_k_cache, B_v_cache, B_wq, B_wo)
```
